```python
import os as _os
_os.environ.setdefault("JAX_PLATFORMS", "cpu")
import jax
import jax.numpy as jnp

def _softmax(x, axis=-1):
    return jax.nn.softmax(x, axis=axis)
def _gelu(x):
    return jax.nn.gelu(x, approximate=True)
def _silu(x):
    return jax.nn.silu(x)
def _sigmoid(x):
    return jax.nn.sigmoid(x)
def _layernorm(x, axis=-1, eps=1e-5):
    m = jnp.mean(x, axis=axis, keepdims=True)
    v = jnp.var(x, axis=axis, keepdims=True)
    return (x - m) / jnp.sqrt(v + eps)
def _scatter_add(tgt, idx, src, axis=0):
    return tgt.at[idx].add(src)
def _segment_sum(src, seg, n):
    return jax.ops.segment_sum(src, seg, n)
class _Rng:
    def __init__(self, key):
        self._k = key
    def _next(self):
        self._k, sub = jax.random.split(self._k)
        return sub
    def normal(self, shape):
        return jax.random.normal(self._next(), shape, dtype=jnp.bfloat16)
    def randint(self, lo, hi, shape):
        return jax.random.randint(self._next(), shape, lo, hi, dtype=jnp.int32)
    def uniform(self, shape, lo=0.0, hi=1.0):
        return jax.random.uniform(self._next(), shape, jnp.bfloat16, lo, hi)
    def permutation(self, n):
        return jax.random.permutation(self._next(), n)


kernel_name = 'standalone__linear_kernel_rfa__decode'

def setup_inputs():
    _rng = _Rng(jax.random.key(int.from_bytes(__import__("os").urandom(4), "little")))
    _w = (lambda a: (lambda t: t.astype(jnp.bfloat16) if jnp.issubdtype(t.dtype, jnp.floating) else t)(jnp.asarray(a)))
    B, H, Sq, Sk, D, M = 2, 16, 1, 16384, 256, 16
    return {
        "q": _w((lambda *s: _rng.normal(s) * 0.4)(B, H, Sq, D)),
        "k": _w((lambda *s: _rng.normal(s) * 1.6)(B, H, Sk, D)),
        "v": _w((lambda *s: _rng.normal(s) * 1.6)(B, H, Sk, D)),
        "omega": _w((lambda *s: _rng.normal(s) * 1.6)(M, D)),
    }

def reference(q, k, v, omega):
    d = q.shape[-1]
    m = omega.shape[0]
    scale = float(d) ** -0.25
    qs = q * scale
    ks = k * scale
    q_proj = jnp.einsum("bhsd,md->bhsm", qs, omega)
    k_proj = jnp.einsum("bhsd,md->bhsm", ks, omega)
    q_sq = 0.5 * jnp.einsum("bhsd,bhsd->bhs", qs, qs)[..., None]
    k_sq = 0.5 * jnp.einsum("bhsd,bhsd->bhs", ks, ks)[..., None]
    inv_sqrt_m = float(m) ** -0.5
    phi_q = jnp.exp(q_proj - q_sq) * inv_sqrt_m + 1e-6
    phi_k = jnp.exp(k_proj - k_sq) * inv_sqrt_m + 1e-6
    kv = jnp.einsum("bhsm,bhsd->bhmd", phi_k, v)
    z  = jnp.einsum("bhsm->bhm", phi_k)
    num = jnp.einsum("bhqm,bhmd->bhqd", phi_q, kv)
    den = jnp.einsum("bhqm,bhm->bhq", phi_q, z)[..., None] + 1e-6
    return num / den
```

```python
import jax, jax.numpy as jnp
from jax import lax
from jax.experimental import pallas as pl
from jax.experimental.pallas import tpu as pltpu

NT = (((1,), (1,)), ((), ()))

def make(ts=1024, L=2, NB=3, taper=(768, 256), piece=64):
    assert sum(taper) == ts
    def kern(q_hbm, k_hbm, v_hbm, om_hbm, o_ref, kbuf, vbuf, qbuf, ombuf, qf, wbuf, phiq, zacc, den, acc, obuf,
             ksem, vsem, tsem, ssem):
        R, D = k_hbm.shape
        M = om_hbm.shape[0]
        BH = q_hbm.shape[0]
        S = R // BH
        cph = S // ts
        n = R // ts
        scale = float(D) ** -0.25
        c = float(M) ** -0.5
        NP = L + 1

        class Multi:
            def __init__(self, hbm, buf, sem, t, off, size, prio):
                self.a = (hbm, buf, sem, t, off, size, prio)
            def pieces(self):
                hbm, buf, sem, t, off, size, prio = self.a
                base = t * ts if isinstance(t, int) else pl.multiple_of(t * ts, ts)
                slot = t % NB
                return [pltpu.make_async_copy(hbm.at[pl.ds(base + off + p * piece, piece)],
                                              buf.at[slot, pl.ds(off + p * piece, piece)], sem) for p in range(size // piece)]
            def start(self):
                for c_ in self.pieces(): c_.start(priority=self.a[6])
            def wait(self):
                hbm, buf, sem, t, off, size, prio = self.a
                dst = buf.at[t % NB, pl.ds(off, size)]
                pltpu.make_async_copy(dst, dst, sem).wait()
        def kcopy(t):
            return Multi(k_hbm, kbuf, ksem.at[t % NB], t, 0, ts, 0)
        def vcopy(t):
            return Multi(v_hbm, vbuf, vsem.at[t % NB], t, 0, ts, 1)
        offs = [sum(taper[:i]) for i in range(len(taper))]
        def vtail(p):
            return Multi(v_hbm, vbuf, tsem.at[p], n - 1, offs[p], taper[p], 1)
        def start2(a, b):
            pa, pb = a.pieces(), b.pieces()
            for x, y in zip(pa, pb):
                x.start(priority=0); y.start(priority=1)
        omcopy = pltpu.make_async_copy(om_hbm, ombuf, ssem.at[0])
        qcopy = pltpu.make_async_copy(q_hbm, qbuf, ssem.at[1])

        omcopy.start()
        qcopy.start()
        kcopy(0).start()
        for t in range(1, NB - 1):
            kcopy(t).start()
            if t - L >= 0:
                vcopy(t - L).start()

        def issue(t):
            tk = t + NB - 1
            tv = tk - L
            if isinstance(t, int):
                if tk < n:
                    kcopy(tk).start()
                if 0 <= tv < n - 1:
                    vcopy(tv).start()
                elif tv == n - 1:
                    for p in range(len(taper)):
                        vtail(p).start()
            else:
                start2(kcopy(tk), vcopy(tv))

        zacc[...] = jnp.zeros_like(zacc)
        acc[...] = jnp.zeros_like(acc)
        omcopy.wait()
        qcopy.wait()
        qf[...] = qbuf[...].astype(jnp.float32) * scale
        ones = jnp.ones((M, 128), jnp.bfloat16)

        def head_start(h):
            q = qf[pl.ds(h, 1), :]
            omf = ombuf[...].astype(jnp.float32)
            qproj = jnp.sum(omf * q, axis=1, keepdims=True)
            qsq = 0.5 * jnp.sum(q * q, axis=1, keepdims=True)
            phiq[...] = jnp.exp(qproj - qsq) * c + 1e-6

        def kstep(t):
            static = isinstance(t, int)
            h = t // cph
            first = (t % cph) == 0
            last = (t % cph) == cph - 1
            if static:
                if first: head_start(h)
            else:
                pl.when(first)(lambda: head_start(h))
            kcopy(t).wait()
            k = kbuf[t % NB]
            kf = k.astype(jnp.float32)
            sq = kf * kf
            sqh = (sq[:, :128] + sq[:, 128:]).astype(jnp.bfloat16)
            om = ombuf[...]
            proj = lax.dot_general(om, k, NT, preferred_element_type=jnp.float32)
            ssq = lax.dot_general(ones, sqh, NT, preferred_element_type=jnp.float32)
            a = proj * scale - ssq * (0.5 * scale * scale)
            phi = jnp.exp(a) * c + 1e-6
            w = jnp.sum(phi * phiq[...], axis=0, keepdims=True)
            wb = jnp.broadcast_to(w, (16, ts)).astype(jnp.bfloat16)
            wbuf[t % NP] = wb
            pf = wb[0:8].astype(jnp.float32)
            zp = pf[:, 0:128]
            for i in range(1, ts // 128):
                zp = zp + pf[:, i * 128:(i + 1) * 128]
            if static:
                z = zp if first else zacc[...] + zp
            else:
                z = jnp.where(first, 0.0, zacc[...]) + zp
            zacc[...] = z
            def fin():
                den[h % 2] = jnp.sum(z, axis=1, keepdims=True) + 1e-6
            if static:
                if last: fin()
            else:
                pl.when(last)(fin)

        def finalize(h, a):
            obuf[pl.ds(h, 1), :] = a[0:1, :] / den[h % 2][0:1, :]

        def vstep(t):
            vcopy(t).wait()
            v = vbuf[t % NB]
            w = wbuf[t % NP]
            part = jnp.dot(w, v, preferred_element_type=jnp.float32)[0:8]
            first = (t % cph) == 0
            if isinstance(t, int):
                a = part if first else acc[...] + part
                acc[...] = a
                if t % cph == cph - 1:
                    finalize(t // cph, a)
            else:
                a = jnp.where(first, 0.0, acc[...]) + part
                acc[...] = a
                @pl.when(t % cph == cph - 1)
                def _():
                    finalize(t // cph, a)

        for t in range(L):
            issue(t)
            kstep(t)
        t_main_end = n - NB + 1
        def body(t, carry):
            issue(t)
            kstep(t)
            vstep(t - L)
            return carry
        lax.fori_loop(L, t_main_end, body, 0)
        for t in range(t_main_end, n + L):
            issue(t)
            if t < n:
                kstep(t)
            tv = t - L
            if tv < n - 1:
                vstep(tv)
            else:
                a = acc[...]
                for p in range(len(taper)):
                    vtail(p).wait()
                    v = vbuf[tv % NB, pl.ds(offs[p], taper[p]), :]
                    w = wbuf[tv % NP, :, pl.ds(offs[p], taper[p])]
                    a = a + jnp.dot(w, v, preferred_element_type=jnp.float32)[0:8]
                finalize(BH - 1, a)
                o_ref[...] = obuf[...].astype(o_ref.dtype)

    @jax.jit
    def f(q, k, v, omega):
        B,H,S,D = k.shape
        M = omega.shape[0]
        q2 = q.reshape(B*H, D)
        k2 = k.reshape(B*H*S, D); v2 = v.reshape(B*H*S, D)
        out = pl.pallas_call(
            kern,
            in_specs=[pl.BlockSpec(memory_space=pl.ANY)]*4,
            out_specs=pl.BlockSpec(memory_space=pltpu.VMEM),
            out_shape=jax.ShapeDtypeStruct((B*H, D), jnp.bfloat16),
            scratch_shapes=[pltpu.VMEM((NB, ts, D), jnp.bfloat16), pltpu.VMEM((NB, ts, D), jnp.bfloat16),
                            pltpu.VMEM((B*H, D), jnp.bfloat16), pltpu.VMEM((M, D), jnp.bfloat16),
                            pltpu.VMEM((B*H, D), jnp.float32),
                            pltpu.VMEM((L+1, 16, ts), jnp.bfloat16),
                            pltpu.VMEM((M, 1), jnp.float32),
                            pltpu.VMEM((8, 128), jnp.float32), pltpu.VMEM((2, 8, 1), jnp.float32),
                            pltpu.VMEM((8, D), jnp.float32), pltpu.VMEM((B*H, D), jnp.float32),
                            pltpu.SemaphoreType.DMA((NB,)), pltpu.SemaphoreType.DMA((NB,)),
                            pltpu.SemaphoreType.DMA((len(taper),)), pltpu.SemaphoreType.DMA((2,))],
            compiler_params=pltpu.CompilerParams(vmem_limit_bytes=64*1024*1024),
        )(q2, k2, v2, omega)
        return out.reshape(B,H,1,D)
    return f


_impl = make(ts=1024, L=2, NB=4, taper=(768, 256), piece=64)


@jax.jit
def pallas_standalone__linear_kernel_rfa__decode_kernel(q, k, v, omega):
    return _impl(q, k, v, omega)
```

```python
import math

import jax
import jax.numpy as jnp
import numpy as np
from jax import lax
from jax.experimental import pallas as pl
from jax.experimental.pallas import tpu as pltpu

_NT = (((1,), (1,)), ((), ()))
_F32 = jnp.float32
_BF16 = jnp.bfloat16

_TS = 1024
_PIECE = 64
_NBUF = 4
_LEAD = 2
_TAPER = (768, 256)


def _rb(x):
    return x.astype(_BF16).astype(_F32)


def _bf16_const(x):
    return float(np.asarray(x, dtype=_BF16))


def _kernel(q_hbm, k_hbm, v_hbm, om_hbm, o_ref,
            kbuf, vbuf, qbuf, ombuf, qf, pbuf, phiq, zacc, den, acc, obuf,
            ksem, vsem, tsem, ssem):
    ts, piece, nb, lead = _TS, _PIECE, _NBUF, _LEAD
    npb = lead + 1
    rows, d = k_hbm.shape
    m = om_hbm.shape[0]
    bh = q_hbm.shape[0]
    cph = rows // bh // ts
    n = rows // ts
    hd = d // 2
    scale = _bf16_const(float(d) ** -0.25)
    fold_scale = math.log2(scale) == round(math.log2(scale))
    post = scale if fold_scale else 1.0
    c = _bf16_const(float(m) ** -0.5)
    eps = _bf16_const(1e-6)
    offs = [sum(_TAPER[:i]) for i in range(len(_TAPER))]

    def pieces(hbm, buf, sem, t, off, size):
        base = t * ts if isinstance(t, int) else pl.multiple_of(t * ts, ts)
        return [pltpu.make_async_copy(hbm.at[pl.ds(base + off + p * piece, piece)],
                                      buf.at[t % nb, pl.ds(off + p * piece, piece)], sem)
                for p in range(size // piece)]

    def wait_all(buf, sem, t, off, size):
        dst = buf.at[t % nb, pl.ds(off, size)]
        pltpu.make_async_copy(dst, dst, sem).wait()

    def k_pieces(t):
        return pieces(k_hbm, kbuf, ksem.at[t % nb], t, 0, ts)

    def v_pieces(t):
        return pieces(v_hbm, vbuf, vsem.at[t % nb], t, 0, ts)

    def v_tail_pieces():
        out = []
        for i, size in enumerate(_TAPER):
            out += pieces(v_hbm, vbuf, tsem.at[i], n - 1, offs[i], size)
        return out

    def start(q0, q1):
        for i in range(max(len(q0), len(q1))):
            if i < len(q0):
                q0[i].start(priority=0)
            if i < len(q1):
                q1[i].start(priority=1)

    def issue(tk):
        tv = tk - lead
        if not isinstance(tk, int):
            start(k_pieces(tk), v_pieces(tv))
            return
        ks = k_pieces(tk) if tk < n else []
        vs = v_pieces(tv) if 0 <= tv < n - 1 else (v_tail_pieces() if tv == n - 1 else [])
        if ks and vs:
            start(ks, vs)
        else:
            both = ks + vs
            start(both[0::2], both[1::2])

    om_copy = pltpu.make_async_copy(om_hbm, ombuf, ssem.at[0])
    q_copy = pltpu.make_async_copy(q_hbm, qbuf, ssem.at[1])
    om_copy.start()
    q_copy.start()
    for t in range(nb - 1):
        issue(t)

    zacc[...] = jnp.zeros_like(zacc)
    acc[...] = jnp.zeros_like(acc)
    om_copy.wait()
    q_copy.wait()
    qf[...] = _rb(qbuf[...].astype(_F32) * scale)
    ones = jnp.ones((m, d), _BF16)

    def feature(proj, ssq):
        a = _rb(_rb(proj) - 0.5 * _rb(ssq))
        return (_rb(_rb(jnp.exp(a)) * c) + eps).astype(_BF16)

    def head_start(h):
        q = qf[pl.ds(h, 1), :]
        qproj = jnp.sum(ombuf[...].astype(_F32) * q, axis=1, keepdims=True)
        qsq = jnp.sum(q * q, axis=1, keepdims=True)
        phiq[h % 2] = feature(qproj, qsq).astype(_F32)

    def k_step(t):
        static = isinstance(t, int)
        h = t // cph
        first = (t % cph) == 0
        last = (t % cph) == cph - 1
        if static:
            if first:
                head_start(h)
        else:
            pl.when(first)(lambda: head_start(h))
        wait_all(kbuf, ksem.at[t % nb], t, 0, ts)
        k = kbuf[t % nb]
        kf = k.astype(_F32)
        if not fold_scale:
            k = (kf * scale).astype(_BF16)
            kf = k.astype(_F32)
        sq = kf * kf
        sqh = sq[:, :hd] + sq[:, hd:]
        hi = sqh.astype(_BF16)
        lo = (sqh - hi.astype(_F32)).astype(_BF16)
        hl = jnp.concatenate([hi, lo], axis=1)
        proj = lax.dot_general(ombuf[...], k, _NT, preferred_element_type=_F32)
        ssq = lax.dot_general(ones, hl, _NT, preferred_element_type=_F32)
        phi = feature(proj * post, ssq * (post * post))
        pbuf[t % npb] = phi
        pf = phi.astype(_F32)
        zp = pf[:, 0:128]
        for i in range(1, ts // 128):
            zp = zp + pf[:, i * 128:(i + 1) * 128]
        if static:
            z = zp if first else zacc[...] + zp
        else:
            z = jnp.where(first, 0.0, zacc[...]) + zp
        zacc[...] = z

        def head_end():
            zz = _rb(jnp.sum(z, axis=1, keepdims=True))
            dd = _rb(jnp.sum(phiq[h % 2] * zz, axis=0, keepdims=True))
            den[h % 2] = _rb(dd + eps)

        if static:
            if last:
                head_end()
        else:
            pl.when(last)(head_end)

    def store_result(h, kv):
        num = _rb(jnp.sum(phiq[h % 2] * _rb(kv), axis=0, keepdims=True))
        obuf[pl.ds(h, 1), :] = num / den[h % 2]

    def v_step(t):
        wait_all(vbuf, vsem.at[t % nb], t, 0, ts)
        part = jnp.dot(pbuf[t % npb], vbuf[t % nb], preferred_element_type=_F32)
        first = (t % cph) == 0
        last = (t % cph) == cph - 1
        if isinstance(t, int):
            kv = part if first else acc[...] + part
            acc[...] = kv
            if last:
                store_result(t // cph, kv)
        else:
            kv = jnp.where(first, 0.0, acc[...]) + part
            acc[...] = kv
            pl.when(last)(lambda: store_result(t // cph, kv))

    for t in range(lead):
        issue(t + nb - 1)
        k_step(t)

    main_end = n - nb + 1

    def body(t, carry):
        issue(t + nb - 1)
        k_step(t)
        v_step(t - lead)
        return carry

    lax.fori_loop(lead, main_end, body, 0)

    for t in range(main_end, n + lead):
        issue(t + nb - 1)
        if t < n:
            k_step(t)
        tv = t - lead
        if tv < n - 1:
            v_step(tv)
        else:
            kv = acc[...]
            for i, size in enumerate(_TAPER):
                wait_all(vbuf, tsem.at[i], tv, offs[i], size)
                kv = kv + jnp.dot(pbuf[tv % npb, :, pl.ds(offs[i], size)],
                                  vbuf[tv % nb, pl.ds(offs[i], size), :],
                                  preferred_element_type=_F32)
            store_result(bh - 1, kv)
            o_ref[...] = obuf[...].astype(o_ref.dtype)


@jax.jit
def pallas_standalone__linear_kernel_rfa__decode_kernel(
    q: jax.Array,
    k: jax.Array,
    v: jax.Array,
    omega: jax.Array,
):
    b, h, s, d = k.shape
    m = omega.shape[0]
    assert q.shape == (b, h, 1, d) and v.shape == k.shape
    assert s % _TS == 0 and s // _TS > _LEAD and d % 256 == 0 and sum(_TAPER) == _TS
    bh = b * h
    out = pl.pallas_call(
        _kernel,
        in_specs=[pl.BlockSpec(memory_space=pl.ANY)] * 4,
        out_specs=pl.BlockSpec(memory_space=pltpu.VMEM),
        out_shape=jax.ShapeDtypeStruct((bh, d), q.dtype),
        scratch_shapes=[
            pltpu.VMEM((_NBUF, _TS, d), _BF16),
            pltpu.VMEM((_NBUF, _TS, d), _BF16),
            pltpu.VMEM((bh, d), _BF16),
            pltpu.VMEM((m, d), _BF16),
            pltpu.VMEM((bh, d), _F32),
            pltpu.VMEM((_LEAD + 1, m, _TS), _BF16),
            pltpu.VMEM((2, m, 1), _F32),
            pltpu.VMEM((m, 128), _F32),
            pltpu.VMEM((2, 1, 1), _F32),
            pltpu.VMEM((m, d), _F32),
            pltpu.VMEM((bh, d), _F32),
            pltpu.SemaphoreType.DMA((_NBUF,)),
            pltpu.SemaphoreType.DMA((_NBUF,)),
            pltpu.SemaphoreType.DMA((len(_TAPER),)),
            pltpu.SemaphoreType.DMA((2,)),
        ],
        compiler_params=pltpu.CompilerParams(
            vmem_limit_bytes=32 * 1024 * 1024,
            disable_bounds_checks=True,
        ),
    )(q.reshape(bh, d), k.reshape(bh * s, d), v.reshape(bh * s, d), omega)
    return out.reshape(b, h, 1, d)
```

```python
import math

import jax
import jax.numpy as jnp
import numpy as np
from jax import lax
from jax.experimental import pallas as pl
from jax.experimental.pallas import tpu as pltpu

_NT = (((1,), (1,)), ((), ()))
_F32 = jnp.float32
_BF16 = jnp.bfloat16

_NREG = 4
_TSR = 256
_PIECE = 64
_NBUF = 5
_LEAD = 3
_SPLIT = 128
_SHIFT = 16


def _rb(x):
    return x.astype(_BF16).astype(_F32)


def _bf16_const(x):
    return float(np.asarray(x, dtype=_BF16))


def _kernel(q_hbm, k_hbm, v_hbm, om_hbm, o_ref,
            kbuf, vbuf, qbuf, ombuf, qf, pbuf, phiq, zacc, den, acc, obuf,
            ksem, vsem, tsem, ssem):
    nreg, tsr, piece, nb, lead, split, sh = _NREG, _TSR, _PIECE, _NBUF, _LEAD, _SPLIT, _SHIFT
    depth = nb - 2
    npb = lead + 1
    npr = tsr // piece
    rows, d = k_hbm.shape
    m = om_hbm.shape[0]
    bh = q_hbm.shape[0]
    s = rows // bh
    cps = s // tsr
    n = rows // (tsr * nreg)
    hd = d // 2
    scale = _bf16_const(float(d) ** -0.25)
    fold_scale = math.log2(scale) == round(math.log2(scale))
    post = scale if fold_scale else 1.0
    c = _bf16_const(float(m) ** -0.5)
    eps = _bf16_const(1e-6)

    def base_row(g):
        b = (g // cps) * (nreg * s) + (g % cps) * tsr
        return b if isinstance(g, int) else pl.multiple_of(b, tsr)

    def copy(hbm, buf, sem, src_row, g, j, r, nr):
        return pltpu.make_async_copy(hbm.at[pl.ds(src_row, nr)],
                                     buf.at[g % nb, j, pl.ds(r, nr)], sem)

    def round_copies(hbm, buf, sem, g, b, p, kind):
        out = []
        for j in range(nreg):
            src = b + j * s + sh + p * piece
            if kind == 'full':
                out.append([copy(hbm, buf, sem, src, g, j, p * piece, piece)])
            else:
                cs = [copy(hbm, buf, sem, src, g, j, p * piece, piece - sh)]
                if kind == 'wrap':
                    nxt = b + tsr - s + nreg * s + j * s
                    cs.append(copy(hbm, buf, sem, nxt, g, j, tsr - sh, sh))
                out.append(cs)
        return out

    def wait_rows(buf, sem, g, lo, hi):
        dst = buf.at[g % nb, :, pl.ds(lo, hi - lo)]
        pltpu.make_async_copy(dst, dst, sem).wait()

    def group_rows(g):
        return tsr - sh if (isinstance(g, int) and g == n - 1) else tsr

    def start_round(kr, vr):
        if kr is not None and vr is not None:
            for j in range(nreg):
                for x in kr[j]:
                    x.start(priority=j % 2)
                for x in vr[j]:
                    x.start(priority=1)
        else:
            for j, xs in enumerate(kr if kr is not None else vr):
                for x in xs:
                    x.start(priority=0 if j % 4 == 0 else 1)

    def static_kind(g, p):
        if p < npr - 1:
            return 'full'
        return 'short' if g == n - 1 else ('wrap' if g % cps == cps - 1 else 'full')

    def issue(gk):
        gv = gk - lead
        if isinstance(gk, int):
            has_k, has_v = gk < n, 0 <= gv < n
            if not (has_k or has_v):
                return
            for p in range(npr):
                kr = vr = None
                if has_k:
                    kr = round_copies(k_hbm, kbuf, ksem.at[gk % nb], gk, base_row(gk), p,
                                      static_kind(gk, p))
                if has_v:
                    sem = (vsem.at[gv % nb] if gv < n - 1
                           else tsem.at[0 if p * piece < split else 1])
                    vr = round_copies(v_hbm, vbuf, sem, gv, base_row(gv), p, static_kind(gv, p))
                start_round(kr, vr)
            return
        bk, bv = base_row(gk), base_row(gv)
        ks, vs = ksem.at[gk % nb], vsem.at[gv % nb]

        def go(p, kkind, vkind):
            start_round(round_copies(k_hbm, kbuf, ks, gk, bk, p, kkind),
                        round_copies(v_hbm, vbuf, vs, gv, bv, p, vkind))

        for p in range(npr - 1):
            go(p, 'full', 'full')
        k_wrap = (gk % cps) == cps - 1
        v_wrap = (gv % cps) == cps - 1
        pl.when(jnp.logical_not(jnp.logical_or(k_wrap, v_wrap)))(
            lambda: go(npr - 1, 'full', 'full'))
        pl.when(k_wrap)(lambda: go(npr - 1, 'wrap', 'full'))
        pl.when(v_wrap)(lambda: go(npr - 1, 'full', 'wrap'))

    om_copy = pltpu.make_async_copy(om_hbm, ombuf, ssem.at[0])
    q_copy = pltpu.make_async_copy(q_hbm, qbuf, ssem.at[1])
    om_copy.start()
    q_copy.start()
    for j in range(nreg):
        copy(k_hbm, kbuf, ssem.at[2], j * s, nb - 1, j, tsr - sh, sh).start()
    for j in range(nreg):
        copy(v_hbm, vbuf, ssem.at[3], j * s, nb - 1, j, tsr - sh, sh).start()
    for g in range(depth):
        issue(g)

    zacc[...] = jnp.zeros_like(zacc)
    acc[...] = jnp.zeros_like(acc)
    om_copy.wait()
    q_copy.wait()
    wait_rows(kbuf, ssem.at[2], nb - 1, tsr - sh, tsr)
    wait_rows(vbuf, ssem.at[3], nb - 1, tsr - sh, tsr)
    qf[...] = _rb(qbuf[...].astype(_F32) * scale)
    ones = jnp.ones((m, d), _BF16)

    def chunk(buf, t, j, lo=0, hi=tsr):
        if lo == 0:
            return jnp.concatenate([buf[(t + nb - 1) % nb, j, pl.ds(tsr - sh, sh), :],
                                    buf[t % nb, j, pl.ds(0, hi - sh), :]], axis=0)
        return buf[t % nb, j, pl.ds(lo - sh, hi - lo), :]

    def feature(proj, ssq):
        a = _rb(_rb(proj) - 0.5 * _rb(ssq))
        return (_rb(_rb(jnp.exp(a)) * c) + eps).astype(_BF16)

    def group_start(sg):
        omf = ombuf[...].astype(_F32)
        for j in range(nreg):
            q = qf[pl.ds(sg * nreg + j, 1), :]
            qproj = jnp.sum(omf * q, axis=1, keepdims=True)
            qsq = jnp.sum(q * q, axis=1, keepdims=True)
            phiq[sg % 2, j] = feature(qproj, qsq).astype(_F32)

    def k_step(t):
        static = isinstance(t, int)
        sg = t // cps
        first = (t % cps) == 0
        last = (t % cps) == cps - 1
        if static:
            if first:
                group_start(sg)
        else:
            pl.when(first)(lambda: group_start(sg))
        wait_rows(kbuf, ksem.at[t % nb], t, 0, group_rows(t))
        k = jnp.concatenate([chunk(kbuf, t, j) for j in range(nreg)], axis=0)
        kf = k.astype(_F32)
        if not fold_scale:
            k = (kf * scale).astype(_BF16)
            kf = k.astype(_F32)
        sq = kf * kf
        sqh = sq[:, :hd] + sq[:, hd:]
        hi = sqh.astype(_BF16)
        lo = (sqh - hi.astype(_F32)).astype(_BF16)
        hl = jnp.concatenate([hi, lo], axis=1)
        proj = lax.dot_general(ombuf[...], k, _NT, preferred_element_type=_F32)
        ssq = lax.dot_general(ones, hl, _NT, preferred_element_type=_F32)
        phi = feature(proj * post, ssq * (post * post))
        pbuf[t % npb] = phi
        pf = phi.astype(_F32)
        zs = []
        for j in range(nreg):
            zp = pf[:, j * tsr:j * tsr + 128]
            for i in range(1, tsr // 128):
                zp = zp + pf[:, j * tsr + i * 128:j * tsr + (i + 1) * 128]
            if static:
                z = zp if first else zacc[j] + zp
            else:
                z = jnp.where(first, 0.0, zacc[j]) + zp
            zacc[j] = z
            zs.append(z)

        def group_end():
            for j in range(nreg):
                zz = _rb(jnp.sum(zs[j], axis=1, keepdims=True))
                dd = _rb(jnp.sum(phiq[sg % 2, j] * zz, axis=0, keepdims=True))
                den[sg % 2, j] = _rb(dd + eps)

        if static:
            if last:
                group_end()
        else:
            pl.when(last)(group_end)

    def store_results(sg, kvs):
        for j in range(nreg):
            num = _rb(jnp.sum(phiq[sg % 2, j] * _rb(kvs[j]), axis=0, keepdims=True))
            obuf[pl.ds(sg * nreg + j, 1), :] = num / den[sg % 2, j]

    def v_step(t):
        static = isinstance(t, int)
        first = (t % cps) == 0
        last = (t % cps) == cps - 1
        wait_rows(vbuf, vsem.at[t % nb], t, 0, tsr)
        kvs = []
        for j in range(nreg):
            part = jnp.dot(pbuf[t % npb, :, pl.ds(j * tsr, tsr)], chunk(vbuf, t, j),
                           preferred_element_type=_F32)
            if static:
                kv = part if first else acc[j] + part
            else:
                kv = jnp.where(first, 0.0, acc[j]) + part
            acc[j] = kv
            kvs.append(kv)
        if static:
            if last:
                store_results(t // cps, kvs)
        else:
            pl.when(last)(lambda: store_results(t // cps, kvs))

    for t in range(lead):
        issue(t + depth)
        k_step(t)

    main_end = n - 1 - depth

    def body(t, carry):
        issue(t + depth)
        k_step(t)
        v_step(t - lead)
        return carry

    lax.fori_loop(lead, main_end, body, 0)

    for t in range(main_end, n + lead):
        issue(t + depth)
        if t < n:
            k_step(t)
        tv = t - lead
        if tv < n - 1:
            v_step(tv)
        else:
            kvs = [acc[j] for j in range(nreg)]
            wait_rows(vbuf, tsem.at[0], tv, 0, split)
            for j in range(nreg):
                kvs[j] = kvs[j] + jnp.dot(pbuf[tv % npb, :, pl.ds(j * tsr, split)],
                                          chunk(vbuf, tv, j, 0, split),
                                          preferred_element_type=_F32)
            wait_rows(vbuf, tsem.at[1], tv, split, tsr - sh)
            for j in range(nreg):
                kvs[j] = kvs[j] + jnp.dot(pbuf[tv % npb, :, pl.ds(j * tsr + split, tsr - split)],
                                          chunk(vbuf, tv, j, split, tsr),
                                          preferred_element_type=_F32)
            store_results(tv // cps, kvs)
            o_ref[...] = obuf[...].astype(o_ref.dtype)


@jax.jit
def pallas_standalone__linear_kernel_rfa__decode_kernel(
    q: jax.Array,
    k: jax.Array,
    v: jax.Array,
    omega: jax.Array,
):
    b, h, s, d = k.shape
    m = omega.shape[0]
    bh = b * h
    assert q.shape == (b, h, 1, d) and v.shape == k.shape and d % 256 == 0
    assert bh % _NREG == 0 and s % _TSR == 0 and s // _TSR > _LEAD + _NBUF
    assert _TSR % 128 == 0 and _TSR % _PIECE == 0 and _SPLIT % 128 == 0 and _SPLIT % _PIECE == 0
    assert 0 < _SHIFT < _PIECE and _SHIFT % 16 == 0 and 0 < _SPLIT < _TSR and _LEAD > 0
    out = pl.pallas_call(
        _kernel,
        in_specs=[pl.BlockSpec(memory_space=pl.ANY)] * 4,
        out_specs=pl.BlockSpec(memory_space=pltpu.VMEM),
        out_shape=jax.ShapeDtypeStruct((bh, d), q.dtype),
        scratch_shapes=[
            pltpu.VMEM((_NBUF, _NREG, _TSR, d), _BF16),
            pltpu.VMEM((_NBUF, _NREG, _TSR, d), _BF16),
            pltpu.VMEM((bh, d), _BF16),
            pltpu.VMEM((m, d), _BF16),
            pltpu.VMEM((bh, d), _F32),
            pltpu.VMEM((_LEAD + 1, m, _NREG * _TSR), _BF16),
            pltpu.VMEM((2, _NREG, m, 1), _F32),
            pltpu.VMEM((_NREG, m, 128), _F32),
            pltpu.VMEM((2, _NREG, 1, 1), _F32),
            pltpu.VMEM((_NREG, m, d), _F32),
            pltpu.VMEM((bh, d), _F32),
            pltpu.SemaphoreType.DMA((_NBUF,)),
            pltpu.SemaphoreType.DMA((_NBUF,)),
            pltpu.SemaphoreType.DMA((2,)),
            pltpu.SemaphoreType.DMA((4,)),
        ],
        compiler_params=pltpu.CompilerParams(
            vmem_limit_bytes=32 * 1024 * 1024,
            disable_bounds_checks=True,
        ),
    )(q.reshape(bh, d), k.reshape(bh * s, d), v.reshape(bh * s, d), omega)
    return out.reshape(b, h, 1, d)
```
